```python
import os as _os
_os.environ.setdefault("JAX_PLATFORMS", "cpu")
import jax
import jax.numpy as jnp

def _softmax(x, axis=-1):
    return jax.nn.softmax(x, axis=axis)
def _gelu(x):
    return jax.nn.gelu(x, approximate=True)
def _silu(x):
    return jax.nn.silu(x)
def _sigmoid(x):
    return jax.nn.sigmoid(x)
def _layernorm(x, axis=-1, eps=1e-5):
    m = jnp.mean(x, axis=axis, keepdims=True)
    v = jnp.var(x, axis=axis, keepdims=True)
    return (x - m) / jnp.sqrt(v + eps)
def _scatter_add(tgt, idx, src, axis=0):
    return tgt.at[idx].add(src)
def _segment_sum(src, seg, n):
    return jax.ops.segment_sum(src, seg, n)
class _Rng:
    def __init__(self, key):
        self._k = key
    def _next(self):
        self._k, sub = jax.random.split(self._k)
        return sub
    def normal(self, shape):
        return jax.random.normal(self._next(), shape, dtype=jnp.bfloat16)
    def randint(self, lo, hi, shape):
        return jax.random.randint(self._next(), shape, lo, hi, dtype=jnp.int32)
    def uniform(self, shape, lo=0.0, hi=1.0):
        return jax.random.uniform(self._next(), shape, jnp.bfloat16, lo, hi)
    def permutation(self, n):
        return jax.random.permutation(self._next(), n)


kernel_name = 'gated_mix__sliding_block_cached__mha_block_cached__decode'

def setup_inputs():
    _rng = _Rng(jax.random.key(int.from_bytes(__import__("os").urandom(4), "little")))
    _w = (lambda a: (lambda t: t.astype(jnp.bfloat16) if jnp.issubdtype(t.dtype, jnp.floating) else t)(jnp.asarray(a)))
    def _A_setup():
        B, Sq, D = 2, 1, 640
        Hq, Hkv, Sk, Dh = 32, 32, 4096, 128
        assert Hq % Hkv == 0, (Hq, Hkv)
        return {
            "x": _w((lambda *s: _rng.normal(s) * 0.05)(B, Sq, D)),
            "k_cache": _w((lambda *s: _rng.normal(s) * 3.2)(B, Hkv, Sk, Dh)),
            "v_cache": _w((lambda *s: _rng.normal(s) * 0.05)(B, Hkv, Sk, Dh)),
            "wq": _w((lambda *s: _rng.normal(s) * 3.2)(D, Hq * Dh) * (D ** -0.5)),
            "wo": _w((lambda *s: _rng.normal(s) * 0.05)(Hq * Dh, D) * ((Hq * Dh) ** -0.5)),
        }
    _A_in = _A_setup()

    def _B_setup():
        B, Sq, D = 2, 1, 640
        H, Sk, Dh = 32, 4096, 128
        return {
            "x": _w((lambda *s: _rng.normal(s) * 0.05)(B, Sq, D)),
            "k_cache": _w((lambda *s: _rng.normal(s) * 3.2)(B, H, Sk, Dh)),
            "v_cache": _w((lambda *s: _rng.normal(s) * 0.05)(B, H, Sk, Dh)),
            "wq": _w((lambda *s: _rng.normal(s) * 3.2)(D, H * Dh) * (D ** -0.5)),
            "wo": _w((lambda *s: _rng.normal(s) * 0.05)(H * Dh, D) * ((H * Dh) ** -0.5)),
        }
    _B_in = _B_setup()

    return {
        "A_x": _A_in["x"],
        "A_k_cache": _A_in["k_cache"],
        "A_v_cache": _A_in["v_cache"],
        "A_wq": _A_in["wq"],
        "A_wo": _A_in["wo"],
        "B_x": _B_in["x"],
        "B_k_cache": _B_in["k_cache"],
        "B_v_cache": _B_in["v_cache"],
        "B_wq": _B_in["wq"],
        "B_wo": _B_in["wo"],
        "gate_w": _w((lambda *s: _rng.normal(s) * 0.05)(640) * 16.0),
    }

def reference(A_x, A_k_cache, A_v_cache, A_wq, A_wo, B_x, B_k_cache, B_v_cache, B_wq, B_wo, gate_w):
    def _A_ref(x, k_cache, v_cache, wq, wo):
        B, Sq, D = x.shape
        Hq, Dh = 32, 128
        Hkv, Sk = k_cache.shape[1], k_cache.shape[2]
        W = min(4096, max(256, Sk // 4))
        rep = Hq // Hkv
        q = (lambda x, *d: x.transpose(*d))((x @ wq).reshape(B, Sq, Hq, Dh), 0, 2, 1, 3)
        k = jnp.repeat(k_cache[:, :, Sk - W:, :], rep, axis=1)
        v = jnp.repeat(v_cache[:, :, Sk - W:, :], rep, axis=1)
        scores = jnp.einsum("bhqd,bhkd->bhqk", q, k) * (Dh ** -0.5)
        p = _softmax(scores, axis=-1)
        o = jnp.einsum("bhqk,bhkd->bhqd", p, v)
        return (lambda x, *d: x.transpose(*d))(o, 0, 2, 1, 3).reshape(B, Sq, Hq * Dh) @ wo

    def _B_ref(x, k_cache, v_cache, wq, wo):
        B, Sq, D = x.shape
        H, Dh = 32, 128
        q = (lambda x, *d: x.transpose(*d))((x @ wq).reshape(B, Sq, H, Dh), 0, 2, 1, 3)
        scores = jnp.einsum("bhqd,bhkd->bhqk", q, k_cache) * (Dh ** -0.5)
        p = _softmax(scores, axis=-1)
        o = jnp.einsum("bhqk,bhkd->bhqd", p, v_cache)
        return (lambda x, *d: x.transpose(*d))(o, 0, 2, 1, 3).reshape(B, Sq, H * Dh) @ wo

    x = A_x
    g = _sigmoid((x * gate_w).sum(-1, keepdims=True))
    a = _A_ref(x, A_k_cache, A_v_cache, A_wq, A_wo)
    b = _B_ref(x, B_k_cache, B_v_cache, B_wq, B_wo)
    return g * a + (1 - g) * b
```

```python
import functools
import jax, jax.numpy as jnp
import jax.experimental.pallas as pl
import jax.experimental.pallas.tpu as pltpu

B, H, S, DH, D, W = 2, 32, 4096, 128, 640, 1024
NT = (((1,), (1,)), ((), ()))

def make(nbuf=4):
    def kern(x_hbm, gw_hbm, ak, av, awq, awo, bk, bv, bwq, bwo, o_ref,
             xv, gwv, wq, wo, kb, vb, ka, va, q_s, o_s, wsem, sems):
        cx = pltpu.make_async_copy(x_hbm, xv, wsem.at[4])
        cg = pltpu.make_async_copy(gw_hbm, gwv, wsem.at[5])
        cw = [pltpu.make_async_copy(awq, wq.at[0], wsem.at[0]), pltpu.make_async_copy(bwq, wq.at[1], wsem.at[1]),
              pltpu.make_async_copy(awo, wo.at[0], wsem.at[2]), pltpu.make_async_copy(bwo, wo.at[1], wsem.at[3])]
        def cps(i):
            h, b = i // 2, i % 2
            s = i % nbuf
            return [pltpu.make_async_copy(bk.at[b, h], kb.at[s], sems.at[0, s]),
                    pltpu.make_async_copy(ak.at[b, h, pl.ds(S - W, W)], ka.at[s], sems.at[1, s]),
                    pltpu.make_async_copy(bv.at[b, h], vb.at[s], sems.at[2, s]),
                    pltpu.make_async_copy(av.at[b, h, pl.ds(S - W, W)], va.at[s], sems.at[3, s])]
        cw[0].start(); cx.start(); cg.start(); cw[1].start()
        for i in range(nbuf):
            for c in cps(i): c.start()
        cx.wait(); cg.wait()
        x = xv[...]
        x16 = jnp.concatenate([x, jnp.zeros((14, D), x.dtype)], axis=0)
        for j in range(2):
            cw[j].wait()
            q = jnp.dot(x16, wq[j], preferred_element_type=jnp.float32).astype(jnp.bfloat16)
            for h in range(H):
                q_s[j, h] = q[:, h * DH:(h + 1) * DH]
        row = jax.lax.broadcasted_iota(jnp.int32, (16, DH), 0)
        scale = DH ** -0.5
        def att(q, k_ref, v_ref, ck, cv):
            ck.wait()
            s = jax.lax.dot_general(q, k_ref[...], NT, preferred_element_type=jnp.float32) * scale
            m = jnp.max(s, axis=-1, keepdims=True)
            p = jnp.exp(s - m)
            l = jnp.sum(p, axis=-1, keepdims=True)
            cv.wait()
            o = jnp.dot(p.astype(jnp.bfloat16), v_ref[...], preferred_element_type=jnp.float32)
            return o / l
        o_s[...] = jnp.zeros_like(o_s)
        def body(i, _):
            h, b = i // 2, i % 2
            s = i % nbuf
            c = cps(i)
            ob = att(q_s[1, h], kb.at[s], vb.at[s], c[0], c[2])
            oa = att(q_s[0, h], ka.at[s], va.at[s], c[1], c[3])
            o_s[1, h] = jnp.where(row == b, ob, o_s[1, h])
            o_s[0, h] = jnp.where(row == b, oa, o_s[0, h])
            @pl.when(i + nbuf < B * H)
            def _():
                for cc in cps(i + nbuf): cc.start()
            @pl.when(i + nbuf == B * H)
            def _():
                cw[2].start(); cw[3].start()
            return 0
        jax.lax.fori_loop(0, B * H, body, 0)
        outs = []
        for j in range(2):
            cw[2 + j].wait()
            acc = jnp.zeros((16, D), jnp.float32)
            for h in range(H):
                acc += jnp.dot(o_s[j, h].astype(jnp.bfloat16), wo[j, h * DH:(h + 1) * DH, :], preferred_element_type=jnp.float32)
            outs.append(acc[:2])
        gw = gwv[...].astype(jnp.float32)
        xf = x.astype(jnp.float32)
        t = jnp.zeros((2, 128), jnp.float32)
        for j in range(D // 128):
            t += xf[:, j * 128:(j + 1) * 128] * gw[j:j + 1, :]
        g = jax.nn.sigmoid(jnp.sum(t, axis=-1, keepdims=True))
        o_ref[...] = (g * outs[0] + (1 - g) * outs[1]).astype(o_ref.dtype)

    def f(A_x, A_k_cache, A_v_cache, A_wq, A_wo, B_x, B_k_cache, B_v_cache, B_wq, B_wo, gate_w):
        bf = jnp.bfloat16
        out = pl.pallas_call(
            kern,
            in_specs=[pl.BlockSpec(memory_space=pltpu.HBM)] * 10,
            out_shape=jax.ShapeDtypeStruct((B, D), bf),
            scratch_shapes=[pltpu.VMEM((B, D), bf), pltpu.VMEM((D // 128, 128), bf),
                            pltpu.VMEM((2, D, H * DH), bf), pltpu.VMEM((2, H * DH, D), bf),
                            pltpu.VMEM((nbuf, S, DH), bf), pltpu.VMEM((nbuf, S, DH), bf),
                            pltpu.VMEM((nbuf, W, DH), bf), pltpu.VMEM((nbuf, W, DH), bf),
                            pltpu.VMEM((2, H, 16, DH), bf), pltpu.VMEM((2, H, 16, DH), jnp.float32),
                            pltpu.SemaphoreType.DMA((6,)), pltpu.SemaphoreType.DMA((4, nbuf))],
            compiler_params=pltpu.CompilerParams(vmem_limit_bytes=100 * 2**20),
        )(A_x.reshape(B, D), gate_w.reshape(D // 128, 128), A_k_cache, A_v_cache, A_wq, A_wo, B_k_cache, B_v_cache, B_wq, B_wo)
        return out.reshape(B, 1, D)
    return f


@jax.jit
def pallas_gated_mix__sliding_block_cached__mha_block_cached__decode_kernel(
    A_x, A_k_cache, A_v_cache, A_wq, A_wo, B_x, B_k_cache, B_v_cache, B_wq, B_wo, gate_w):
    return make(2)(A_x, A_k_cache, A_v_cache, A_wq, A_wo, B_x, B_k_cache, B_v_cache, B_wq, B_wo, gate_w)
```

```python
import functools
import jax, jax.numpy as jnp
import numpy as np
import jax.experimental.pallas as pl
import jax.experimental.pallas.tpu as pltpu

B, H, S, DH, D, W = 2, 32, 4096, 128, 640, 1024
NI = B * H
NT = (((1,), (1,)), ((), ()))
C = float(DH ** -0.5 * np.log2(np.e))
bf, f32 = jnp.bfloat16, jnp.float32


def make(R=8, d1=103, d2=45, d2b=35, d3=45, d4=60, d5=70, RK=4, RV=8, fine_bg=False, checks=False, dlast=None, scopes=False,
         fin_batches=((0, 1, 2, 3, 4, 5), ('f', 6), (7, 8), (9,))):
    NFG = 24

    def kern(x_hbm, gw_hbm, ak, av, awq, awo, bk, bv, bwq, bwo, o_ref,
             xv, gwv, wq, wo, kb, vb, ka, va, q_s, o_s, sb, sa,
             xsem, wqsem, ksem, bsem, wofsem, wobsem):
        row = jax.lax.broadcasted_iota(jnp.int32, (R, DH), 0)

        def scope(name):
            import contextlib
            return jax.named_scope(name) if scopes else contextlib.nullcontext()

        def delay(d):
            if d:
                pl.delay(d)

        cx = pltpu.make_async_copy(x_hbm, xv, xsem.at[0])
        cg = pltpu.make_async_copy(gw_hbm, gwv, xsem.at[1])
        c_bwq_tail = pltpu.make_async_copy(bwq.at[pl.ds(512, 128)], wq.at[1, pl.ds(512, 128)], wqsem.at[1])
        c_awq = pltpu.make_async_copy(awq, wq.at[0], wqsem.at[2])

        def c_bwq(n):
            r = pl.multiple_of((n // 2) * 8, 8)
            c = pl.multiple_of((n % 2) * 2048, 2048)
            return pltpu.make_async_copy(bwq.at[pl.ds(r, 8), pl.ds(c, 2048)],
                                         wq.at[1, pl.ds(r, 8), pl.ds(c, 2048)], wqsem.at[0])
        c_bwq_all = pltpu.make_async_copy(wq.at[1, pl.ds(0, 512)], wq.at[1, pl.ds(0, 512)], wqsem.at[0])

        def c_k(i, j):
            r = pl.multiple_of(j * 128, 128)
            return pltpu.make_async_copy(bk.at[i % 2, i // 2, pl.ds(r, 128)], kb.at[i % RK, pl.ds(r, 128)], ksem.at[i % RK])

        def c_k_all(i):
            return pltpu.make_async_copy(kb.at[i % RK], kb.at[i % RK], ksem.at[i % RK])

        def c_bg(i):
            b, h, s = i % 2, i // 2, i % RV
            return [pltpu.make_async_copy(ak.at[b, h, pl.ds(S - W, W)], ka.at[s], bsem.at[s, 0]),
                    pltpu.make_async_copy(av.at[b, h, pl.ds(S - W, W)], va.at[s], bsem.at[s, 1]),
                    pltpu.make_async_copy(bv.at[b, h], vb.at[s], bsem.at[s, 2])]

        def c_bg_fine(c):
            i, g = c // 8, c % 8
            b, h, s = i % 2, i // 2, i % RV
            ra = pl.multiple_of(g * 128, 128)
            rs = pl.multiple_of(S - W + g * 128, 128)
            rb = pl.multiple_of(g * 512, 512)
            sem = bsem.at[c % 16]
            return [pltpu.make_async_copy(ak.at[b, h, pl.ds(rs, 128)], ka.at[s, pl.ds(ra, 128)], sem),
                    pltpu.make_async_copy(av.at[b, h, pl.ds(rs, 128)], va.at[s, pl.ds(ra, 128)], sem),
                    pltpu.make_async_copy(bv.at[b, h, pl.ds(rb, 512)], vb.at[s, pl.ds(rb, 512)], sem)]

        def c_wof(n):
            r = pl.multiple_of(n * 32, 32)
            rr = pl.multiple_of(H * DH + n * 32, 32)
            return pltpu.make_async_copy(bwo.at[pl.ds(r, 32)], wo.at[pl.ds(rr, 32)], wofsem.at[n // 8])

        def c_wof_all(dg):
            rr = pl.multiple_of(H * DH + dg * 256, 256)
            return pltpu.make_async_copy(wo.at[pl.ds(rr, 256)], wo.at[pl.ds(rr, 256)], wofsem.at[dg])

        def c_wob3(dg):
            r = dg * 384
            if not isinstance(r, int):
                r = pl.multiple_of(r, 128)
            return pltpu.make_async_copy(awo.at[pl.ds(r, 384)], wo.at[pl.ds(r, 384)], wobsem.at[dg])
        tail_blocks = [(1, 24), (1, 25), (1, 26), (1, 27), (1, 28), (1, 29), (0, 30), (1, 30), (0, 31), (1, 31)]

        def c_wob1(k):
            br, h = tail_blocks[k]
            src = (awo, bwo)[br]
            return pltpu.make_async_copy(src.at[pl.ds(h * DH, DH)], wo.at[pl.ds((br * H + h) * DH, DH)], wobsem.at[10 + k])

        c_bwq_tail.start(priority=1)
        c_awq.start(priority=1)
        cx.start()
        cg.start()
        if fine_bg:
            for c in range(8):
                for cp in c_bg_fine(c):
                    cp.start(priority=1)
        else:
            for cp in c_bg(0):
                cp.start(priority=1)

        def p1(n, _):
            c_bwq(n).start()
            delay(d1)
            return 0
        with scope('P1'):
            jax.lax.fori_loop(0, 128, p1, 0)

        def bg_top(t, wait=True, start=True):
            if fine_bg:
                return
            if wait:
                for cp in c_bg(t - 1):
                    cp.wait()
            if start:
                for cp in c_bg(t + 1):
                    cp.start(priority=1)

        def bg_group(c, wait=True, start=True):
            if not fine_bg:
                return
            if wait:
                for cp in c_bg_fine(c - 1):
                    cp.wait()
            if start:
                for cp in c_bg_fine(c + 7):
                    cp.start(priority=1)

        bg_top(0, wait=False)
        o_s[...] = jnp.zeros_like(o_s)

        def p2a(g, _):
            @pl.when(g > 0)
            def _():
                bg_group(g)
            for u in range(4):
                c_k(0, 4 * g + u).start()
                delay(d1)
            return 0
        with scope('P2a'):
            jax.lax.fori_loop(0, 8, p2a, 0)

        bg_top(1)
        with scope('Wq_wait'):
            cx.wait(); cg.wait(); c_bwq_all.wait(); c_bwq_tail.wait(); c_awq.wait()
        x = xv[...]
        xp = jnp.concatenate([x, jnp.zeros((R - B, D), bf)], axis=0)
        xf = xp.astype(f32)
        gw = gwv[...].astype(f32)
        t = xf[:, 0:128] * gw[0:1, :]
        for j in range(1, D // 128):
            t += xf[:, j * 128:(j + 1) * 128] * gw[j:j + 1, :]
        gate = jax.nn.sigmoid(jnp.sum(t, axis=-1, keepdims=True))
        gate = jnp.broadcast_to(gate, (R, DH))

        def qproj(n):
            br = (n // 8) % 2
            h = (n // 16) * 16 + (n % 8) * 2
            col = pl.multiple_of(h * DH, 2 * DH)
            q = jnp.dot(xp, wq[br, :, pl.ds(col, 2 * DH)], preferred_element_type=f32).astype(bf)
            q_s[br, h] = q[:, :DH]
            q_s[br, h + 1] = q[:, DH:]

        def p2b(g, _):
            bg_group(8 + g)
            for pr in range(2):
                j = 4 * g + 2 * pr
                c_k(1, j).start()
                qproj(2 * g + pr)
                delay(1)
                c_k(1, j + 1).start()
                delay(d2)
            return 0
        with scope('P2b'):
            jax.lax.fori_loop(0, 8, p2b, 0)

        neg = jnp.full((R, DH), -jnp.inf, f32)
        zero = jnp.zeros((R, DH), f32)

        def iteration(t, mb_prev, ma_prev, acc_out, do_qk, do_pv, do_wo):
            iq, ip = t - 2, t - 3
            par = t % 2
            if do_qk:
                with scope('kwait' + ('e' if do_wo else '')):
                    c_k_all(iq).wait()
                qa, qb = q_s[0, iq // 2], q_s[1, iq // 2]
            if do_pv:
                mb = jnp.broadcast_to(jnp.max(mb_prev, axis=-1, keepdims=True) * C, (R, DH))
                ma = jnp.broadcast_to(jnp.max(ma_prev, axis=-1, keepdims=True) * C, (R, DH))

            def group(g, carry, par2=None):
                mbr, mar, lb, la, accb, acca, acc_out = carry
                if not do_wo:
                    bg_group(8 * t + g)
                ra = pl.multiple_of(g * 128, 128)
                for pr in range(2):
                    js = [4 * g + 2 * pr, 4 * g + 2 * pr + 1]
                    rs = [pl.multiple_of(j * 128, 128) for j in js]

                    def issue(j):
                        if do_wo:
                            c_wof((t - NI) * 32 + j).start()
                        else:
                            c_k(t, j).start()
                    if do_wo:
                        dg = (t - NI) * 4 + g // 2
                        ks = ([2, 3], [4], [0], [1])[par2 * 2 + pr]
                        if 0 in ks:
                            @pl.when(dg >= 1)
                            def _():
                                with scope('wofwait'):
                                    c_wof_all(dg - 1).wait()
                        if 2 in ks:
                            @pl.when(dg >= 2)
                            def _():
                                with scope('wobwait'):
                                    c_wob3(dg - 2).wait()
                    issue(js[0])
                    if not do_pv:
                        qproj(16 + 2 * g + pr)
                    if do_pv:
                        ps = [jnp.exp2(sb[1 - par, j] * C - mb) for j in js]
                        if pr == 1:
                            pa = jnp.exp2(sa[1 - par, g] * C - ma)
                    if do_qk:
                        for j, r in zip(js, rs):
                            s = jax.lax.dot_general(qb, kb[iq % RK, pl.ds(r, 128)], NT, preferred_element_type=f32)
                            sb[par, j] = s
                            mbr = jnp.maximum(mbr, s)
                        if pr == 0:
                            s = jax.lax.dot_general(qa, ka[iq % RV, pl.ds(ra, 128)], NT, preferred_element_type=f32)
                            sa[par, g] = s
                            mar = jnp.maximum(mar, s)
                    if do_pv:
                        for p, r in zip(ps, rs):
                            lb = lb + p
                            accb = accb + jnp.dot(p.astype(bf), vb[ip % RV, pl.ds(r, 128)], preferred_element_type=f32)
                        if pr == 1:
                            la = la + pa
                            acca = acca + jnp.dot(pa.astype(bf), va[ip % RV, pl.ds(ra, 128)], preferred_element_type=f32)
                    if do_wo:
                        for k in ks:
                            if k < 2:
                                idx = H + jnp.maximum(2 * (dg - 1) + k, 0)
                                ok = dg >= 1
                            else:
                                idx = jnp.maximum(3 * (dg - 2) + (k - 2), 0)
                                ok = dg >= 2
                            rr = pl.multiple_of(idx * DH, DH)
                            y = jnp.dot(o_s[idx].astype(bf), wo[pl.ds(rr, DH)], preferred_element_type=f32)
                            acc_out = jnp.where(ok, acc_out + y, acc_out)
                    delay(1)
                    issue(js[1])
                    delay((d4 if do_qk else d5) if do_wo else (d3 if do_pv else d2b))
                return mbr, mar, lb, la, accb, acca, acc_out

            carry = (neg, neg, zero, zero, zero, zero, acc_out)
            if do_wo:
                def dgroup(gg, carry):
                    carry = group(2 * gg, carry, 0)
                    return group(2 * gg + 1, carry, 1)
                carry = jax.lax.fori_loop(0, 4, dgroup, carry)
            else:
                carry = jax.lax.fori_loop(0, 8, group, carry)
            mbr, mar, lb, la, accb, acca, acc_out = carry
            if do_pv:
                b, h = ip % 2, ip // 2
                ob = accb * ((1.0 - gate) / jnp.sum(lb, axis=-1, keepdims=True))
                oa = acca * (gate / jnp.sum(la, axis=-1, keepdims=True))
                o_s[H + h] = jnp.where(row == b, ob, o_s[H + h])
                o_s[h] = jnp.where(row == b, oa, o_s[h])
            return mbr, mar, acc_out

        bg_top(2)
        with scope('T2'):
            mb, ma, _ = iteration(2, None, None, 0, True, False, False)

        def main(t, carry):
            with scope('bgw'):
                bg_top(t)
            mb, ma, _ = iteration(t, carry[0], carry[1], 0, True, True, False)
            return mb, ma
        with scope('Main'):
            mb, ma = jax.lax.fori_loop(3, NI - 1, main, (mb, ma))

        assert not fine_bg
        bg_top(NI - 1, start=False)
        for dg in range(10):
            c_wob3(dg).start(priority=1)
        for k in range(10):
            c_wob1(k).start(priority=1)
        with scope('T63'):
            mb, ma, _ = iteration(NI - 1, mb, ma, 0, True, True, False)

        with scope('bg64'):
            bg_top(NI, start=False)
        acc = jnp.zeros((R, D), f32)

        def endloop(t, carry):
            return iteration(t, carry[0], carry[1], carry[2], True, True, True)
        with scope('End64_65'):
            mb, ma, acc = jax.lax.fori_loop(NI, NI + 2, endloop, (mb, ma, acc))
        with scope('End66'):
            _, _, acc = iteration(NI + 2, mb, ma, acc, False, True, True)

        def outp(acc, idxs):
            lhs = [o_s[i].astype(bf) for i in idxs]
            for i, l in zip(idxs, lhs):
                acc = acc + jnp.dot(l, wo[pl.ds(i * DH, DH)], preferred_element_type=f32)
            return acc
        tb = [br * H + h for br, h in tail_blocks]
        with scope('Fin'):
            for batch in fin_batches:
                idxs = []
                for k in batch:
                    if k == 'f':
                        c_wof_all(11).wait()
                        idxs += [H + 22, H + 23]
                    else:
                        c_wob1(k).wait()
                        idxs.append(tb[k])
                acc = outp(acc, idxs)
        o_ref[...] = acc[:B].astype(o_ref.dtype)

    def f(A_x, A_k_cache, A_v_cache, A_wq, A_wo, B_x, B_k_cache, B_v_cache, B_wq, B_wo, gate_w):
        out = pl.pallas_call(
            kern,
            in_specs=[pl.BlockSpec(memory_space=pltpu.HBM)] * 10,
            out_shape=jax.ShapeDtypeStruct((B, D), bf),
            scratch_shapes=[pltpu.VMEM((B, D), bf), pltpu.VMEM((D // 128, 128), bf),
                            pltpu.VMEM((2, D, H * DH), bf), pltpu.VMEM((2 * H * DH, D), bf),
                            pltpu.VMEM((RK, S, DH), bf), pltpu.VMEM((RV, S, DH), bf),
                            pltpu.VMEM((RV, W, DH), bf), pltpu.VMEM((RV, W, DH), bf),
                            pltpu.VMEM((2, H, R, DH), bf), pltpu.VMEM((2 * H, R, DH), f32),
                            pltpu.VMEM((2, S // 128, R, 128), f32), pltpu.VMEM((2, W // 128, R, 128), f32),
                            pltpu.SemaphoreType.DMA((2,)), pltpu.SemaphoreType.DMA((3,)), pltpu.SemaphoreType.DMA((RK,)),
                            pltpu.SemaphoreType.DMA((16,) if fine_bg else (RV, 3)),
                            pltpu.SemaphoreType.DMA((12,)), pltpu.SemaphoreType.DMA((20,))],
            compiler_params=pltpu.CompilerParams(vmem_limit_bytes=100 * 2**20,
                                                 disable_bounds_checks=not checks, disable_semaphore_checks=not checks),
        )(A_x.reshape(B, D), gate_w.reshape(D // 128, 128), A_k_cache, A_v_cache, A_wq, A_wo, B_k_cache, B_v_cache, B_wq, B_wo)
        return out.reshape(B, 1, D)
    return f


@jax.jit
def pallas_gated_mix__sliding_block_cached__mha_block_cached__decode_kernel(
    A_x, A_k_cache, A_v_cache, A_wq, A_wo, B_x, B_k_cache, B_v_cache, B_wq, B_wo, gate_w):
    return make(d2=35,d2b=25,d4=40,d5=50)(A_x, A_k_cache, A_v_cache, A_wq, A_wo, B_x, B_k_cache, B_v_cache, B_wq, B_wo, gate_w)
```

```python
import contextlib
import jax, jax.numpy as jnp
import numpy as np
import jax.experimental.pallas as pl
import jax.experimental.pallas.tpu as pltpu

B, H, S, DH, D, W = 2, 32, 4096, 128, 640, 1024
NI = B * H
NT = (((1,), (1,)), ((), ()))
C = float(DH ** -0.5 * np.log2(np.e))
bf, f32 = jnp.bfloat16, jnp.float32
G = 256
R = 8


def mo(x, m):
    return x if isinstance(x, int) else pl.multiple_of(x, m)


def make(off=192, a=64, gap=17, gapq=17, g1=10, g2=6, gapw=0, dp1=133, dq0=130, dq=10, dx=40, QL=20, dm=127, db=1, dw0=100, dw=0, RV=8,
         checks=False, nocomp=0, scopes=False, XV=5,
         fin=(('a26', 'a27'), ('b28', 'b29'), ('a28', 'a29'), ('b30', 'b31'), ('a30',), ('a31',))):
    KA0 = NI * S
    VA0 = RV * S
    c0 = off * 16
    T0 = off // 8

    def kern(x_hbm, gw_hbm, ak, av, awq, awo, bk, bv, bwq, bwo, o_ref,
             xv, gwv, x_s, wq, wo, kb, vb, q_s, o_s, s_s, st_s,
             xsem, wqsem, ksem, vsem, bsem, wofsem, wobsem):
        row = jax.lax.broadcasted_iota(jnp.int32, (R, DH), 0)

        def scope(name):
            return jax.named_scope(name) if scopes else contextlib.nullcontext()

        def delay(d):
            if d:
                pl.delay(d)

        def copy(src, dst, sem):
            return pltpu.make_async_copy(src, dst, sem)

        cx = copy(x_hbm, xv, xsem.at[0])
        cg = copy(gw_hbm, gwv, xsem.at[1])

        def c_awq(kb_):
            r = mo(kb_ * 128, 128)
            return copy(awq.at[pl.ds(r, 128)], wq.at[0, pl.ds(r, 128)], wqsem.at[0, kb_])

        def c_bwq_all(kb_):
            r = mo(kb_ * 128, 128)
            return copy(wq.at[1, pl.ds(r, 128)], wq.at[1, pl.ds(r, 128)], wqsem.at[1, kb_])

        def c_bwq(rg, lo, hi):
            r = mo(rg * 8, 8)
            return copy(bwq.at[pl.ds(r, 8), pl.ds(lo, hi - lo)], wq.at[1, pl.ds(r, 8), pl.ds(lo, hi - lo)], wqsem.at[1, rg // 16])

        def c_k(i, r, n):
            r = mo(i * S + r, 8)
            return copy(bk.at[pl.ds(r, n)], kb.at[pl.ds(r, n)], ksem.at[i % 4])

        def c_k_all(i, n=S):
            r = mo(i * S + off, 8)
            return copy(kb.at[pl.ds(r, n)], kb.at[pl.ds(r, n)], ksem.at[i % 4])
        c_k_head = copy(bk.at[pl.ds(0, off)], kb.at[pl.ds(0, off)], xsem.at[2])

        def c_v(i, r, n):
            return copy(bv.at[pl.ds(mo(i * S + r, 8), n)], vb.at[pl.ds(mo((i % RV) * S + r, 8), n)], vsem.at[i % 4])

        def c_v_all(i):
            r = mo((i % RV) * S + off, 8)
            return copy(vb.at[pl.ds(r, XV * G)], vb.at[pl.ds(r, XV * G)], vsem.at[i % 4])

        def c_bg(i):
            s = i % RV
            ra = mo(i * S + (S - W), W)
            lo = off + XV * G
            return [copy(bv.at[pl.ds(mo(i * S, S), off)], vb.at[pl.ds(mo(s * S, S), off)], bsem.at[s, 0]),
                    copy(ak.at[pl.ds(ra, W)], kb.at[pl.ds(mo(KA0 + s * W, W), W)], bsem.at[s, 1]),
                    copy(av.at[pl.ds(ra, W)], vb.at[pl.ds(mo(VA0 + s * W, W), W)], bsem.at[s, 2]),
                    copy(bv.at[pl.ds(mo(i * S + lo, 8), S - lo)], vb.at[pl.ds(mo(s * S + lo, 8), S - lo)], bsem.at[s, 3])]

        def c_wo_tiles(rnd, t0, t1):
            out = []
            while t0 < t1:
                rg, c = divmod(t0, 5)
                if c or t1 - t0 < 5:
                    n = min(5 - c, t1 - t0)
                    nr, lo, nc = 8, c * 128, n * 128
                else:
                    n = (t1 - t0) // 5 * 5
                    nr, lo, nc = n // 5 * 8, 0, D
                r = mo(rnd * 512 + rg * 8, 8)
                out.append(copy(bwo.at[pl.ds(r, nr), pl.ds(lo, nc)],
                                wo.at[pl.ds(mo(H * DH + r, 8), nr), pl.ds(lo, nc)], wofsem.at[rnd]))
                t0 += n
            return out

        def c_awo(h, n):
            r = mo(h * DH, DH)
            return copy(awo.at[pl.ds(r, n * DH)], wo.at[pl.ds(r, n * DH)], wobsem.at[h // 2 if n == 2 else h - 15])

        def group(first, rest, g):
            first.start()
            delay(g)
            for cp in rest:
                cp.start()

        def k_group(t, g, last=False):
            r = off + g * G
            if last:
                c_k(t, r, G - off).start()
            else:
                group(c_k(t, r, a), [c_k(t, r + a, G - a)], gap)

        def v_group(t, g):
            r = off + g * G
            group(c_v(t, r, a), [c_v(t, r + a, G - a)], gap)

        def kv_group(t, g, may_be_last=False, gp=None):
            is_k, is_v = g < 16, g >= 16
            rk, rv = off + g * G, off + (g - 16) * G
            last = jnp.logical_and(t == NI - 1, g == 15) if may_be_last else False

            @pl.when(is_k)
            def _():
                c_k(t, rk, a).start()

            @pl.when(is_v)
            def _():
                c_v(t, rv, a).start()
            delay(gap if gp is None else gp)

            @pl.when(jnp.logical_and(is_k, jnp.logical_not(last)) if may_be_last else is_k)
            def _():
                c_k(t, rk + a, G - a).start()
            if may_be_last and G - off - a > 0:
                @pl.when(last)
                def _():
                    c_k(t, rk + a, G - off - a).start()

            @pl.when(is_v)
            def _():
                c_v(t, rv + a, G - a).start()

        for k in range(D // 128):
            c_awq(k).start(priority=1)
            if k == 0:
                c_bwq(0, 0, c0).start()
                cx.start()
                cg.start()
        for cp in c_bg(0):
            cp.start(priority=1)

        def wq_group(n):
            group(c_bwq(n, c0, H * DH), [c_bwq(n + 1, 0, c0)], gapq)

        def p1a(n, _):
            wq_group(n)
            delay(dp1)
            return 0
        with scope('P1a'):
            jax.lax.fori_loop(0, QL - 1, p1a, 0)
        wq_group(QL - 1)
        for cp in c_bg(1):
            cp.start(priority=1)
        q_s[...] = jnp.zeros_like(q_s)
        cx.wait()
        cg.wait()
        xp = jnp.concatenate([xv[...], jnp.zeros((R - B, D), bf)], axis=0)
        for k in range(D // 128):
            x_s[k] = xp[:, k * 128:(k + 1) * 128]
        delay(dx)

        def q_wait(n):
            @pl.when(n % 16 == 0)
            def _():
                c_awq(n // 16).wait()
                c_bwq_all(n // 16).wait()

        def q_unit(n):
            k, br, c = n // 16, (n // 8) % 2, n % 8
            y = jnp.dot(x_s[k], wq[br, pl.ds(mo(k * 128, 128), 128), pl.ds(mo(c * 512, 512), 512)], preferred_element_type=f32)
            for i in range(4):
                q_s[br * H + 4 * c + i] += y[:, i * DH:(i + 1) * DH]

        def p1b(n, _):
            q_wait(n - QL)
            wq_group(n)
            q_unit(n - QL)
            delay(dq)
            return 0
        with scope('P1b'):
            jax.lax.fori_loop(QL, D // 8 - 1, p1b, 0)
        group(c_bwq(D // 8 - 1, c0, H * DH), [c_k_head], gapq)
        o_s[...] = jnp.zeros_like(o_s)
        s_s[...] = jnp.zeros_like(s_s)
        st_s[...] = jnp.zeros_like(st_s)
        delay(dx)

        def t0(g, _):
            n = D // 8 - 1 - QL + g
            q_wait(n)
            kv_group(0, g)
            q_unit(n)
            delay(dq)
            return 0
        with scope('T0'):
            jax.lax.fori_loop(0, QL + 1, t0, 0)
        assert QL + 1 == 16 + XV
        for cp in c_bg(0):
            cp.wait()
        for cp in c_bg(2):
            cp.start(priority=1)
        c_k_head.wait()

        def t1(g, _):
            kv_group(1, g)
            delay(dq0)
            return 0
        with scope('T1'):
            jax.lax.fori_loop(0, 16 + XV - 1, t1, 0)
        kv_group(1, 16 + XV - 1)
        xf = xp.astype(f32)
        gw = gwv[...].astype(f32)
        t = xf[:, 0:128] * gw[0:1, :]
        for j in range(1, D // 128):
            t += xf[:, j * 128:(j + 1) * 128] * gw[j:j + 1, :]
        gate = jax.nn.sigmoid(jnp.sum(t, axis=-1, keepdims=True))
        gate = jnp.broadcast_to(gate, (R, DH))
        delay(db)

        neg = jnp.full((R, DH), -jnp.inf, f32)
        zero = jnp.zeros((R, DH), f32)

        def attend(iq, ip, par, j, carry):
            mrun, l, acc = carry
            isa = j >= 8
            br = jnp.where(isa, 0, 1)
            fresh = jnp.logical_or(j == 0, j == 8)
            mrun = jnp.where(fresh, neg, mrun)
            l = jnp.where(fresh, zero, l)
            acc = jnp.where(fresh, zero, acc)
            kr = jnp.where(isa, KA0 + (iq % RV) * W + (j - 8) * 512, iq * S + j * 512)
            vr = jnp.where(isa, VA0 + (ip % RV) * W + (j - 8) * 512, (ip % RV) * S + j * 512)
            q = q_s[br * H + iq % H].astype(bf)
            m = st_s[3 * br]
            ps = [jnp.exp2(s_s[1 - par, 4 * j + u] * C - m) for u in range(4)]
            for u in range(4):
                s = jax.lax.dot_general(q, kb[pl.ds(mo(kr + u * 128, 128), 128)], NT, preferred_element_type=f32)
                s_s[par, 4 * j + u] = s
                mrun = jnp.maximum(mrun, s)
            for u in range(4):
                l = l + ps[u]
                acc = acc + jnp.dot(ps[u].astype(bf), vb[pl.ds(mo(vr + u * 128, 128), 128)], preferred_element_type=f32)
            st_s[6 + br] = mrun
            st_s[3 * br + 1] = l
            st_s[3 * br + 2] = acc
            return mrun, l, acc

        def boundary(ip, store=True):
            b, h = ip // H, ip % H
            for br, wgt in ((0, gate), (1, 1.0 - gate)):
                o = st_s[3 * br + 2] * (wgt / jnp.sum(st_s[3 * br + 1], axis=-1, keepdims=True))
                keep = row == b if store is True else jnp.logical_and(row == b, store)
                o_s[br * H + h] = jnp.where(keep, o, o_s[br * H + h])
                st_s[3 * br] = jnp.broadcast_to(jnp.max(st_s[6 + br], axis=-1, keepdims=True) * C, (R, DH))

        def main(t, _):
            iq, ip, par = t - 2, jnp.maximum(t - 3, 0), t % 2
            with scope('bgw'):
                for cp in c_bg(t - 1):
                    cp.wait()

            @pl.when(t < NI - 1)
            def _():
                for cp in c_bg(t + 1):
                    cp.start(priority=1)

            @pl.when(t == NI - 1)
            def _():
                for h in range(0, 30, 2):
                    c_awo(h, 2).start(priority=1)
                c_awo(30, 1).start(priority=1)
                c_awo(31, 1).start(priority=1)
            with scope('kw'):
                c_k_all(iq).wait()
                c_v_all(iq).wait()

            def dp(j, carry):
                kv_group(t, 2 * j, gp=g1)
                if nocomp:
                    delay(nocomp)
                else:
                    carry = attend(iq, ip, par, j, carry)
                delay(1)
                kv_group(t, 2 * j + 1, True, gp=g2)
                delay(dm)
                return carry
            jax.lax.fori_loop(0, 10, dp, (neg, zero, zero))
            if XV == 5:
                v_group(t, 4)
            boundary(ip)
            delay(db)
            return 0
        with scope('Main'):
            jax.lax.fori_loop(2, NI, main, 0)

        for cp in c_bg(NI - 1):
            cp.wait()
        for cp in c_wo_tiles(0, 0, T0):
            cp.start()

        def outp(acc, idxs):
            for i in idxs:
                acc = acc + jnp.dot(o_s[i].astype(bf), wo[pl.ds(mo(i * DH, DH), DH)], preferred_element_type=f32)
            return acc

        def wait_wof(rnd, lo, hi):
            for cp in c_wo_tiles(rnd, lo, hi):
                cp.wait()

        def wo_round(r, carry):
            att, out = carry[:3], carry[3]
            t = NI + r // 2
            iq, ip, par = jnp.minimum(t - 2, NI - 1), jnp.minimum(t - 3, NI - 1), t % 2

            @pl.when(r == 0)
            def _():
                c_k_all(NI - 2).wait()
                c_v_all(NI - 2).wait()

            @pl.when(r == 2)
            def _():
                c_k_all(NI - 1, S - off).wait()
                c_v_all(NI - 1).wait()
            for d in range(5):
                for half in range(2):
                    k = 2 * d + half
                    lo, hi = T0 + 32 * k, T0 + 32 * (k + 1)
                    if hi <= 320:
                        cps = c_wo_tiles(r, lo, hi)
                        group(cps[0], cps[1:], gapw)
                    else:
                        cps = c_wo_tiles(r, lo, 320)
                        group(cps[0], cps[1:], gapw)

                        @pl.when(r < 7)
                        def _():
                            for cp in c_wo_tiles(r + 1, 0, T0):
                                cp.start()
                    if half == 0:
                        att = attend(iq, ip, par, 5 * (r % 2) + d, att)
                        delay(1)
                    elif d == 0:
                        delay(dw0)
                    else:
                        if d == 1:
                            @pl.when(r >= 1)
                            def _():
                                r0 = mo(H * DH + (r - 1) * 512, 512)
                                copy(wo.at[pl.ds(r0, 512)], wo.at[pl.ds(r0, 512)], wofsem.at[r - 1]).wait()
                        if d < 3:
                            h = 4 * (r - 1) + 2 * (d - 1)
                            base = H
                        else:
                            h = 4 * (r - 1) + 2 * (d - 3) - 2
                            base = 0

                            @pl.when(h >= 0)
                            def _():
                                c_awo(h, 2).wait()
                        ok = h >= 0
                        hc = jnp.maximum(h, 0)

                        new = outp(out, [base + hc, base + hc + 1])
                        out = jnp.where(ok, new, out)
                        delay(dw)

            @pl.when(r % 2 == 1)
            def _():
                boundary(ip, store=t - 3 < NI)
            return (*att, out)
        with scope('Wo'):
            carry = jax.lax.fori_loop(0, 8, wo_round, (neg, zero, zero, jnp.zeros((R, D), f32)))
        out = carry[3]

        with scope('Fin'):
            waited_b = False
            for batch in fin:
                idxs = []
                for name in batch:
                    h = int(name[1:])
                    if name[0] == 'b':
                        if not waited_b:
                            r0 = H * DH + 7 * 512
                            copy(wo.at[pl.ds(r0, 512)], wo.at[pl.ds(r0, 512)], wofsem.at[7]).wait()
                            waited_b = True
                        idxs.append(H + h)
                    else:
                        if h >= 30:
                            c_awo(h, 1).wait()
                        elif h % 2 == 0:
                            c_awo(h, 2).wait()
                        idxs.append(h)
                out = outp(out, idxs)
        o_ref[...] = out[:B].astype(o_ref.dtype)

    def f(A_x, A_k_cache, A_v_cache, A_wq, A_wo, B_x, B_k_cache, B_v_cache, B_wq, B_wo, gate_w):
        flat = lambda c: c.reshape(NI * S, DH)
        out = pl.pallas_call(
            kern,
            in_specs=[pl.BlockSpec(memory_space=pltpu.HBM)] * 10,
            out_shape=jax.ShapeDtypeStruct((B, D), bf),
            scratch_shapes=[pltpu.VMEM((B, D), bf), pltpu.VMEM((D // 128, 128), bf), pltpu.VMEM((D // 128, R, 128), bf),
                            pltpu.VMEM((2, D, H * DH), bf), pltpu.VMEM((2 * H * DH, D), bf),
                            pltpu.VMEM((NI * S + RV * W, DH), bf), pltpu.VMEM((RV * (S + W), DH), bf),
                            pltpu.VMEM((2 * H, R, DH), f32), pltpu.VMEM((2 * H, R, DH), f32),
                            pltpu.VMEM((2, (S + W) // 128, R, 128), f32), pltpu.VMEM((8, R, 128), f32),
                            pltpu.SemaphoreType.DMA((3,)), pltpu.SemaphoreType.DMA((2, D // 128)),
                            pltpu.SemaphoreType.DMA((4,)), pltpu.SemaphoreType.DMA((4,)),
                            pltpu.SemaphoreType.DMA((RV, 4)),
                            pltpu.SemaphoreType.DMA((8,)), pltpu.SemaphoreType.DMA((17,))],
            compiler_params=pltpu.CompilerParams(vmem_limit_bytes=110 * 2**20,
                                                 disable_bounds_checks=not checks, disable_semaphore_checks=not checks),
        )(A_x.reshape(B, D), gate_w.reshape(D // 128, 128), flat(A_k_cache), flat(A_v_cache), A_wq, A_wo,
          flat(B_k_cache), flat(B_v_cache), B_wq, B_wo)
        return out.reshape(B, 1, D)
    return f


@jax.jit
def pallas_gated_mix__sliding_block_cached__mha_block_cached__decode_kernel(
    A_x, A_k_cache, A_v_cache, A_wq, A_wo, B_x, B_k_cache, B_v_cache, B_wq, B_wo, gate_w):
    return make()(A_x, A_k_cache, A_v_cache, A_wq, A_wo, B_x, B_k_cache, B_v_cache, B_wq, B_wo, gate_w)
```

```python
import jax
import jax.numpy as jnp
import numpy as np
import jax.experimental.pallas as pl
import jax.experimental.pallas.tpu as pltpu

B, H, S, DH, D = 2, 32, 4096, 128, 640
W = min(4096, max(256, S // 4))
ITEMS = B * H
A, BR_B = 0, 1
ROWS = 8
TILE = 128
SCALE = float(DH ** -0.5 * np.log2(np.e))

GROUP = 256
LEAD = 16
PHASE_A, PHASE_B = 128, 192
RING = 4
WO_TILES = H * DH // 8 * (D // TILE)
HEAD_TILES = WO_TILES // H
Q_LAG = 21
VA_BASE = ITEMS * S
V_ZERO = VA_BASE + RING * W

PAUSE = dict(
    lead=15, start=107, wq=219, gate=7, q=45, zero=3, q_item=48, q_two=7,
    qk=13, pv=38, qk6=18, pv6=39, qk7=18, pv7=46, qk8=11, pv8=34, qk9=18, pv9=27,
    wo_qk=3, wo_pv=37, wo_qk8=19, wo_pv8=51, wo_qk9=19, wo_pv9=51,
    one=39, pv_one=5, one_x=42, pv_one_x=19, one_y=45, pv_one_y=19,
    two=7, second=43, last0=221, last1=39, last2=6,
)

bf16, f32 = jnp.bfloat16, jnp.float32


def _multiple_of(x, m):
    return x if isinstance(x, int) else pl.multiple_of(x, m)


def _pause(kind):
    pl.delay(-(-2 * PAUSE[kind] // 3))


def _dot(a, b):
    return jnp.dot(a, b, preferred_element_type=f32)


def _wait_all(ref, sem):
    pltpu.make_async_copy(ref, ref, sem).wait()


def _wait(copies):
    for copy in copies:
        copy.wait()


def _start_if(cond, make_copies, priority=0):
    def start():
        for copy in make_copies():
            copy.start(priority=priority)

    if cond is True:
        start()
    elif cond is not False:
        pl.when(cond)(start)


def _start_period(lead, rest, low):
    lead.start()
    _pause("lead")
    for copy in rest:
        copy.start()
    pl.delay(1)
    for copy in low:
        copy.start(priority=1)


def _kernel(x_hbm, gw_hbm, ak_hbm, av_hbm, awq_hbm, awo_hbm, bk_hbm, bv_hbm, bwq_hbm, bwo_hbm,
            o_ref,
            x_ref, gw_ref, xk_ref, wq_ref, wo_ref, kb_ref, ka_ref, v_ref,
            q_ref, att_ref, s_ref, out_ref,
            misc_sem, wq_sem, kb_sem, ka_sem, vb_sem, va_sem, wo_sem):
    copy = pltpu.make_async_copy
    row = jax.lax.broadcasted_iota(jnp.int32, (ROWS, DH), 0)

    def wq_copy(br, rg, lo, hi):
        r = pl.ds(_multiple_of(rg * 8, 8), 8)
        c = pl.ds(lo, hi - lo)
        return copy((awq_hbm, bwq_hbm)[br].at[r, c], wq_ref.at[br, r, c], wq_sem.at[br, rg >> 4])

    def kb_copy(i, r, n):
        slot = i & (RING - 1)
        return copy(bk_hbm.at[pl.ds(_multiple_of(i * S + r, 8), n)],
                    kb_ref.at[slot, pl.ds(_multiple_of(r, 8), n)], kb_sem.at[slot])

    def vb_copy(i, r, n):
        rows = pl.ds(_multiple_of(i * S + r, 8), n)
        return copy(bv_hbm.at[rows], v_ref.at[rows], vb_sem.at[i & (RING - 1)])

    def vb_wait(i, n=S):
        _wait_all(v_ref.at[pl.ds(_multiple_of(i * S + PHASE_B, 8), n)], vb_sem.at[i & (RING - 1)])

    def window_pieces(g):
        if g < 3:
            return [(PHASE_A + g * GROUP, GROUP)]
        return [(PHASE_A + 3 * GROUP, GROUP - PHASE_A), (0, PHASE_A)]

    def ka_copies(i, g):
        slot = i & (RING - 1)
        return [copy(ak_hbm.at[pl.ds(_multiple_of(i * S + S - W + r, 8), n)],
                     ka_ref.at[slot, pl.ds(r, n)], ka_sem.at[int(g == 0), slot])
                for r, n in window_pieces(g)]

    def va_copies(i, g):
        slot = i & (RING - 1)
        return [copy(av_hbm.at[pl.ds(_multiple_of(i * S + S - W + r, 8), n)],
                     v_ref.at[pl.ds(_multiple_of(VA_BASE + slot * W + r, 8), n)], va_sem.at[slot])
                for r, n in window_pieces(g)]

    def va_wait(i):
        slot = i & (RING - 1)
        _wait_all(v_ref.at[pl.ds(_multiple_of(VA_BASE + slot * W, W), W)], va_sem.at[slot])

    def wo_copy(br, t0, n, m):
        return copy((awo_hbm, bwo_hbm)[br].at[pl.ds(t0, n)],
                    wo_ref.at[pl.ds(br * WO_TILES + t0, n)], wo_sem.at[br, m])

    def item_period(t, p, part):
        more = t < ITEMS - 1
        if isinstance(p, int) and p == 18:
            _wait(ka_copies(t, 0))
        if part < 2:
            r = PHASE_B + p * GROUP
            kb_copy(t, r, LEAD).start()
            _pause("lead")
            edge = p == 15 if part == 1 else False
            _start_if(p < 15 if part == 1 else True, lambda: [kb_copy(t, r + LEAD, GROUP - LEAD)])
            _start_if(edge, lambda: [kb_copy(t, PHASE_B + 15 * GROUP + LEAD, GROUP - PHASE_B - LEAD)])
            _start_if(edge if edge is False else edge & more, lambda: [kb_copy(t + 1, 0, PHASE_B)])
        else:
            r = PHASE_B + (p - 16) * GROUP
            vb_copy(t, r, LEAD).start()
            _pause("lead")
            vb_copy(t, r + LEAD, GROUP - LEAD).start()
        pl.delay(1)
        if part == 0:
            full = more if isinstance(more, bool) else (p < 11) | more
            _start_if(full, lambda: [vb_copy(t, PHASE_B + (p + 4) * GROUP, GROUP)], 1)
            _start_if(False if full is True else jnp.logical_not(full),
                      lambda: [vb_copy(t, PHASE_B + 15 * GROUP, GROUP - PHASE_B)], 1)
        else:
            copies = ka_copies if part == 1 else va_copies
            for g in range(4):
                _start_if(p - (12 if part == 1 else 16) == g, lambda: copies(t, g), 1)

    col_a, col_b, col_lead = PHASE_A * 16, PHASE_B * 16, LEAD * 16
    x_copy = copy(x_hbm, x_ref, misc_sem.at[0])
    gw_copy = copy(gw_hbm, gw_ref, misc_sem.at[1])
    v_first = copy(bv_hbm.at[pl.ds(0, PHASE_B)], v_ref.at[pl.ds(0, PHASE_B)], misc_sem.at[2])
    wq_copy(BR_B, 0, 0, col_b).start()
    wq_copy(A, 0, 0, col_a).start(priority=1)
    x_copy.start()
    gw_copy.start()
    _pause("start")

    def wq_period(n, next_high=None, next_low=None):
        _start_period(wq_copy(BR_B, n, col_b, col_b + col_lead),
                      [wq_copy(BR_B, n, col_b + col_lead, H * DH), next_high or wq_copy(BR_B, n + 1, 0, col_b)],
                      [wq_copy(A, n, col_a, H * DH), next_low or wq_copy(A, n + 1, 0, col_a)])

    def wq_only(n, _):
        wq_period(n)
        _pause("wq")

    jax.lax.fori_loop(0, Q_LAG - 1, wq_only, None)

    wq_period(Q_LAG - 1)
    q_ref[...] = jnp.zeros_like(q_ref)
    x_copy.wait()
    gw_copy.wait()
    x = jnp.concatenate([x_ref[...], jnp.zeros((ROWS - B, D), bf16)], axis=0)
    for k in range(D // TILE):
        xk_ref[k] = x[:, k * TILE:(k + 1) * TILE]
    xf = x.astype(f32)
    gw = gw_ref[...].astype(f32)
    logit = xf[:, :TILE] * gw[:1]
    for k in range(1, D // TILE):
        logit += xf[:, k * TILE:(k + 1) * TILE] * gw[k:k + 1]
    gate = jax.nn.sigmoid(jnp.sum(logit, axis=-1, keepdims=True))
    gate = jnp.broadcast_to(gate, (ROWS, DH))
    _pause("gate")

    def q_wait(n):
        @pl.when(n & 15 == 0)
        def _():
            k = n >> 4
            for br in range(2):
                _wait_all(wq_ref.at[br, pl.ds(_multiple_of(k * TILE, TILE), TILE)], wq_sem.at[br, k])

    def q_unit(n):
        k, br, c = n >> 4, (n >> 3) & 1, n & 7
        y = _dot(xk_ref[k], wq_ref[br, pl.ds(_multiple_of(k * TILE, TILE), TILE),
                                   pl.ds(_multiple_of(c * 4 * DH, 4 * DH), 4 * DH)])
        for i in range(4):
            q_ref[br * H + 4 * c + i] += y[:, i * DH:(i + 1) * DH]

    def wq_and_q(n, _):
        q_wait(n - Q_LAG)
        wq_period(n)
        q_unit(n - Q_LAG)
        _pause("q")

    last = D // 8 - 1
    jax.lax.fori_loop(Q_LAG, last, wq_and_q, None)

    wq_period(last, kb_copy(0, 0, PHASE_B), v_first)
    q_unit(last - Q_LAG)
    att_ref[...] = jnp.zeros_like(att_ref)
    s_ref[...] = jnp.zeros_like(s_ref)
    v_ref[pl.ds(V_ZERO, 4 * TILE)] = jnp.zeros((4 * TILE, DH), bf16)
    _pause("zero")

    def first_item(p, part, two=False):
        n = last + 1 - Q_LAG + p
        if part == 0:
            q_wait(n)
        item_period(0, p, part)
        if two:
            q_unit(2 * p + 40)
            q_unit(2 * p + 41)
        else:
            q_unit(n)
        _pause("q_two" if two else "q_item")

    jax.lax.fori_loop(0, 12, lambda p, _: first_item(p, 0), None)
    jax.lax.fori_loop(12, 16, lambda p, _: first_item(p, 1), None)
    jax.lax.fori_loop(16, 40 - Q_LAG, lambda p, _: first_item(p, 2), None)
    jax.lax.fori_loop(40 - Q_LAG, 20, lambda p, _: first_item(p, 2, True), None)
    _wait(ka_copies(0, 0))
    v_first.wait()

    neg_inf = jnp.full((ROWS, DH), -jnp.inf, f32)
    zero = jnp.zeros((ROWS, DH), f32)

    def scores(i, par, j, in_a, run_max):
        q = q_ref[(0 if in_a else H) + (i & (H - 1))].astype(bf16)
        for u in range(4):
            if in_a:
                k = ka_ref[i & (RING - 1), pl.ds((j - 8) * 4 * TILE + u * TILE, TILE)]
            else:
                k = kb_ref[i & (RING - 1), pl.ds(_multiple_of(j * 4 * TILE + u * TILE, TILE), TILE)]
            s = jax.lax.dot_general(q, k, (((1,), (1,)), ((), ())), preferred_element_type=f32)
            s_ref[par, 4 * j + u] = s
            run_max = jnp.maximum(run_max, s)
        return run_max

    def weighted_values(i, par, j, in_a, shift, total, acc):
        r = VA_BASE + (i & (RING - 1)) * W + (j - 8) * 4 * TILE if in_a else i * S + j * 4 * TILE
        r = jnp.where(i < 0, V_ZERO, r)
        for u in range(4):
            p = jnp.exp2(s_ref[1 - par, 4 * j + u] * SCALE - shift)
            total = total + p
            acc = acc + _dot(p.astype(bf16), v_ref[pl.ds(_multiple_of(r + u * TILE, TILE), TILE)])
        return total, acc

    def softmax_shift(run_max):
        return jnp.broadcast_to(jnp.max(run_max, axis=-1, keepdims=True) * SCALE, (ROWS, DH))

    def finish(br, i, total, acc):
        i = jnp.maximum(i, 0)
        o = acc * ((gate if br == A else 1.0 - gate) / jnp.sum(total, axis=-1, keepdims=True))
        h = br * H + (i & (H - 1))
        att_ref[h] = jnp.where(row == (i >> 5), o, att_ref[h])

    def data_wait(t):
        slot = (t - 1) & (RING - 1)
        _wait_all(kb_ref.at[slot], kb_sem.at[slot])
        for g in range(1, 4):
            _wait(ka_copies(t - 1, g))

        @pl.when(t - 2 >= 0)
        def _():
            vb_wait(t - 2)
            va_wait(t - 2)

    def attend(t, carry, issue, prefix, rolled):
        shift_b, max_a, total_a, acc_a = carry
        iq, ip, par = t - 1, t - 2, t & 1

        def step(j, state, part, tag):
            run_max, total, acc = state
            shift = None
            issue(2 * j, part)
            run_max = scores(iq, par, j, part == 2, run_max)
            if tag == "7":
                shift = softmax_shift(max_a)
            if tag == "9":
                shift = softmax_shift(state_b[0])
            _pause(prefix + "qk" + tag)
            issue(2 * j + 1, part)
            total, acc = weighted_values(ip, par, j, part == 2, shift_a if part == 2 else shift_b, total, acc)
            if tag == "6":
                finish(A, ip - 1, total_a, acc_a)
            if tag == "8":
                finish(BR_B, ip, state_b[1], state_b[2])
            _pause(prefix + "pv" + tag)
            return (run_max, total, acc), shift

        state = jax.lax.fori_loop(0, rolled, lambda j, st: step(j, st, 0, "")[0], (neg_inf, zero, zero))
        if rolled == 6:
            state, _ = step(6, state, 1, "6")
            state_b, shift_a = step(7, state, 1, "7")
        else:
            state_b = state
            finish(A, ip - 1, total_a, acc_a)
            shift_a = softmax_shift(max_a)
        state, _ = step(8, (neg_inf, zero, zero), 2, "8")
        state, shift_b = step(9, state, 2, "9")
        return (shift_b, *state)

    def item(t, carry):
        data_wait(t)
        return attend(t, carry, lambda p, part: item_period(t, p, part), "", 6)

    carry = jax.lax.fori_loop(1, ITEMS, item, (zero, zero, zero + 1.0, zero))

    tile_a, tile_b, tile_lead = PHASE_A // 8, PHASE_B // 8, LEAD // 8
    quad = 4 * HEAD_TILES
    last_groups = ((28, 2, 7), (30, 1, 8), (31, 1, 9))
    wo_copy(BR_B, 0, tile_b, 0).start()
    wo_copy(A, 0, tile_a, 0).start(priority=1)

    def tenth(n):
        return (n * 205) >> 11

    def wo_period(p):
        m = tenth(p)
        k = p - m * 10
        t0 = p * 32
        wo_copy(BR_B, t0 + tile_b, tile_lead, m).start()
        _pause("lead")

        @pl.when(k < 9)
        def _():
            wo_copy(BR_B, t0 + tile_b + tile_lead, 32 - tile_lead, m).start()

        @pl.when(k == 9)
        def _():
            wo_copy(BR_B, t0 + tile_b + tile_lead, 32 - tile_b - tile_lead, m).start()
            wo_copy(BR_B, t0 + 32, tile_b, m + 1).start()

        pl.delay(1)

        @pl.when(k < 9)
        def _():
            wo_copy(A, t0 + tile_a, 32, m).start(priority=1)

        @pl.when(k == 9)
        def _():
            wo_copy(A, t0 + tile_a, 32 - tile_a, m).start(priority=1)
            wo_copy(A, t0 + 32, tile_a, m + 1).start(priority=1)

    def last_pieces(t0):
        pieces = []
        for h, n, m in last_groups:
            lo, hi = max(t0, h * HEAD_TILES), min(t0 + 32, (h + n) * HEAD_TILES)
            if lo < hi:
                pieces.append((lo, hi - lo, m))
        return pieces

    def wo_last_period(k):
        t0 = 7 * quad + 32 * k
        (lo, n, m), *others = last_pieces(t0 + tile_b)
        rest = [(lo + tile_lead, n - tile_lead, m), *others]
        _start_period(wo_copy(BR_B, lo, tile_lead, m),
                      [wo_copy(BR_B, *piece) for piece in rest if piece[1]],
                      [wo_copy(A, *piece) for piece in last_pieces(t0 + tile_a)])

    def out_wait(u):
        @pl.when(jnp.asarray(u - tenth(u) * 10 == 0))
        def _():
            m = tenth(u)
            for br in range(2):
                _wait_all(wo_ref.at[pl.ds(br * WO_TILES + m * quad, quad)], wo_sem.at[br, m])

    def out_unit(u):
        m = tenth(u)
        k = u - m * 10
        br = jnp.where(k >= 5, 1, 0)
        c = k - 5 * br
        acc = out_ref[c]
        for i in range(4):
            h = br * H + 4 * m + i
            w = jnp.concatenate([wo_ref[h * HEAD_TILES + c + 5 * r] for r in range(16)], axis=0)
            acc = acc + _dot(att_ref[h].astype(bf16), w)
        out_ref[c] = acc

    def out_heads(heads):
        out = [out_ref[c] for c in range(5)]
        for br in range(2):
            for h in heads:
                o = att_ref[br * H + h].astype(bf16)
                w = wo_ref[pl.ds((br * H + h) * HEAD_TILES, HEAD_TILES)].reshape(16, 5, 8, TILE)
                for c in range(5):
                    out[c] = out[c] + _dot(o, w[:, c].reshape(TILE, TILE))
        return out

    def heads_wait(h, n, m):
        for br in range(2):
            _wait_all(wo_ref.at[pl.ds(br * WO_TILES + h * HEAD_TILES, n * HEAD_TILES)], wo_sem.at[br, m])

    out_ref[...] = jnp.zeros_like(out_ref)
    data_wait(ITEMS)
    shift_b, max_a, total_a, acc_a = attend(ITEMS, carry, lambda p, part: wo_period(p), "wo_", 8)

    vb_wait(ITEMS - 1, S - PHASE_B)
    va_wait(ITEMS - 1)

    def last_item_step(j, state, in_a, shift, tag, also=None):
        out_wait(2 * j)
        wo_period(20 + 2 * j)
        out_unit(2 * j)
        result = also() if also else None
        _pause("one" + tag)
        wo_period(21 + 2 * j)
        state = weighted_values(ITEMS - 1, (ITEMS + 1) & 1, j, in_a, shift, *state)
        out_unit(2 * j + 1)
        _pause("pv_one" + tag)
        return state, result

    def next_to_last_a():
        finish(A, ITEMS - 2, total_a, acc_a)
        return softmax_shift(max_a)

    state = jax.lax.fori_loop(0, 7, lambda j, st: last_item_step(j, st, False, shift_b, "")[0], (zero, zero))
    state_b, shift_a = last_item_step(7, state, False, shift_b, "_x", next_to_last_a)
    state, _ = last_item_step(8, (zero, zero), True, shift_a, "_x", lambda: finish(BR_B, ITEMS - 1, *state_b))
    state, _ = last_item_step(9, state, True, shift_a, "_y")

    def out_period(issue, p, units, kind, also=None):
        for u in units:
            out_wait(u)
        issue(p)
        for u in units:
            out_unit(u)
        if also:
            also()
        _pause(kind)

    def two_units(e, also=None):
        out_period(wo_period, 2 * e, [2 * e - 20], "one", also)
        out_period(wo_period, 2 * e + 1, [2 * e - 19], "second")

    def three_units(e):
        out_period(wo_period, 2 * e, [3 * e - 50, 3 * e - 49], "two")
        out_period(wo_period, 2 * e + 1, [3 * e - 48], "second")

    two_units(20, lambda: finish(A, ITEMS - 1, *state))
    jax.lax.fori_loop(21, 30, lambda e, _: two_units(e), None)
    jax.lax.fori_loop(30, 35, lambda e, _: three_units(e), None)
    u = 55
    for k, n in enumerate((2, 2, 1, 0, 2, 2, 2, 2, 2)):
        out_period(wo_last_period, k, range(u, u + n), "last%d" % n)
        u += n

    for h, n, m in last_groups:
        heads_wait(h, n, m)
        if h == 28:
            wo_last_period(9)
        out = out_heads(range(h, h + n))
        if h < H - 1:
            for c in range(5):
                out_ref[c] = out[c]
    for c in range(5):
        o_ref[:, c * TILE:(c + 1) * TILE] = out[c][:B].astype(o_ref.dtype)


@jax.jit
def pallas_gated_mix__sliding_block_cached__mha_block_cached__decode_kernel(
    A_x: jax.Array,
    A_k_cache: jax.Array,
    A_v_cache: jax.Array,
    A_wq: jax.Array,
    A_wo: jax.Array,
    B_x: jax.Array,
    B_k_cache: jax.Array,
    B_v_cache: jax.Array,
    B_wq: jax.Array,
    B_wo: jax.Array,
    gate_w: jax.Array,
):
    del B_x

    def rows(cache):
        return cache.reshape(ITEMS * S, DH)

    def tiles(wo):
        return wo.reshape(H * DH // 8, 8, D // TILE, TILE).transpose(0, 2, 1, 3).reshape(WO_TILES, 8, TILE)

    dma = pltpu.SemaphoreType.DMA
    out = pl.pallas_call(
        _kernel,
        in_specs=[pl.BlockSpec(memory_space=pltpu.HBM)] * 10,
        out_shape=jax.ShapeDtypeStruct((B, D), bf16),
        scratch_shapes=[
            pltpu.VMEM((B, D), bf16),
            pltpu.VMEM((D // TILE, TILE), bf16),
            pltpu.VMEM((D // TILE, ROWS, TILE), bf16),
            pltpu.VMEM((2, D, H * DH), bf16),
            pltpu.VMEM((2 * WO_TILES, 8, TILE), bf16),
            pltpu.VMEM((RING, S, DH), bf16),
            pltpu.VMEM((RING, W, DH), bf16),
            pltpu.VMEM((V_ZERO + 4 * TILE, DH), bf16),
            pltpu.VMEM((2 * H, ROWS, DH), f32),
            pltpu.VMEM((2 * H, ROWS, DH), f32),
            pltpu.VMEM((2, (S + W) // TILE, ROWS, TILE), f32),
            pltpu.VMEM((D // TILE, ROWS, TILE), f32),
            dma((3,)), dma((2, D // TILE)), dma((RING,)), dma((2, RING)),
            dma((RING,)), dma((RING,)), dma((2, 10)),
        ],
        compiler_params=pltpu.CompilerParams(
            vmem_limit_bytes=110 * 2**20,
            disable_bounds_checks=True,
            disable_semaphore_checks=True,
        ),
    )(A_x.reshape(B, D), gate_w.reshape(D // TILE, TILE),
      rows(A_k_cache), rows(A_v_cache), A_wq, tiles(A_wo),
      rows(B_k_cache), rows(B_v_cache), B_wq, tiles(B_wo))
    return out.reshape(B, 1, D)
```
